```python
import jax
import jax.numpy as jnp

def _softmax(x, axis=-1):
    return jax.nn.softmax(x, axis=axis)

def _gelu(x):
    return jax.nn.gelu(x, approximate=True)

def _silu(x):
    return jax.nn.silu(x)

def _sigmoid(x):
    return jax.nn.sigmoid(x)

def _layernorm(x, axis=-1, eps=1e-05):
    m = jnp.mean(x, axis=axis, keepdims=True)
    v = jnp.var(x, axis=axis, keepdims=True)
    return (x - m) / jnp.sqrt(v + eps)

def _scatter_add(tgt, idx, src, axis=0):
    return tgt.at[idx].add(src)

def _segment_sum(src, seg, n):
    return jax.ops.segment_sum(src, seg, n)

class _Rng:

    def __init__(self, key):
        self._k = key

    def _next(self):
        self._k, sub = jax.random.split(self._k)
        return sub

    def normal(self, shape):
        return jax.random.normal(self._next(), shape, dtype=jnp.bfloat16)

    def randint(self, lo, hi, shape):
        return jax.random.randint(self._next(), shape, lo, hi, dtype=jnp.int32)

    def uniform(self, shape, lo=0.0, hi=1.0):
        return jax.random.uniform(self._next(), shape, jnp.bfloat16, lo, hi)

    def permutation(self, n):
        return jax.random.permutation(self._next(), n)
kernel_name = 'concat_heads__compressed_kv_cla__memory_aug_recurrent_mem_tr__prompt'

def setup_inputs():
    _rng = _Rng(jax.random.key(int.from_bytes(__import__("os").urandom(4), "little")))
    _w = lambda a: (lambda t: t.astype(jnp.bfloat16) if jnp.issubdtype(t.dtype, jnp.floating) else t)(jnp.asarray(a))

    def _A_setup():
        B, H, Sq, Sk, D, M = (1, 32, 2048, 2048, 128, 576)
        Dc = 4 * D
        return {'x': _w((lambda *s: _rng.normal(s) * 0.05)(B, Sq, M)), 'c_kv': _w((lambda *s: _rng.normal(s) * 0.05)(B, Sk, Dc)), 'w_q': _w((lambda *s: _rng.normal(s) * 0.05)(M, H, D) * M ** (-0.5)), 'w_uk': _w((lambda *s: _rng.normal(s) * 0.05)(Dc, H, D) * Dc ** (-0.5)), 'w_uv': _w((lambda *s: _rng.normal(s) * 0.05)(Dc, H, D) * Dc ** (-0.5)), 'w_o': _w((lambda *s: _rng.normal(s) * 0.05)(H, D, M) * (H * D) ** (-0.5))}
    _A_in = _A_setup()

    def _B_setup():
        B, S, Dm = (1, 2048, 576)
        H, Dh = (32, 128)
        M, seg = (8, 32)
        seg = min(seg, S)
        S = S // seg * seg
        return {'x': _w((lambda *s: _rng.normal(s) * 0.05)(B, S, Dm)), 'mem0': _w((lambda *s: _rng.normal(s) * 0.05)(B, M, Dm)), 'Wq': _w((lambda *s: _rng.normal(s) * 0.05)(Dm, H, Dh) * Dm ** (-0.5)), 'Wk': _w((lambda *s: _rng.normal(s) * 0.05)(Dm, H, Dh) * Dm ** (-0.5)), 'Wv': _w((lambda *s: _rng.normal(s) * 0.05)(Dm, H, Dh) * Dm ** (-0.5)), 'Wo': _w((lambda *s: _rng.normal(s) * 0.05)(H, Dh, Dm) * (H * Dh) ** (-0.5)), 'seg_len': seg}
    _B_in = _B_setup()
    return {'A_x': _A_in['x'], 'A_c_kv': _A_in['c_kv'], 'A_w_q': _A_in['w_q'], 'A_w_uk': _A_in['w_uk'], 'A_w_uv': _A_in['w_uv'], 'A_w_o': _A_in['w_o'], 'B_x': _B_in['x'], 'B_mem0': _B_in['mem0'], 'B_Wq': _B_in['Wq'], 'B_Wk': _B_in['Wk'], 'B_Wv': _B_in['Wv'], 'B_Wo': _B_in['Wo'], 'B_seg_len': _B_in['seg_len']}

def reference(A_x, A_c_kv, A_w_q, A_w_uk, A_w_uv, A_w_o, B_x, B_mem0, B_Wq, B_Wk, B_Wv, B_Wo, B_seg_len):

    def _A_ref(x, c_kv, w_q, w_uk, w_uv, w_o):
        B, Sq, M = (x.shape[0], x.shape[1], x.shape[2])
        Sk = c_kv.shape[1]
        H, D = (w_q.shape[1], w_q.shape[2])
        q = jnp.einsum('bqm,mhd->bhqd', x, w_q)
        k = jnp.einsum('bkc,chd->bhkd', c_kv, w_uk)
        v = jnp.einsum('bkc,chd->bhkd', c_kv, w_uv)
        scores = jnp.einsum('bhqd,bhkd->bhqk', q, k) * D ** (-0.5)
        off = Sk - Sq
        qi = jnp.arange(Sq)[:, None]
        kj = jnp.arange(Sk)[None, :]
        cmask = kj <= qi + off
        scores = jnp.where(cmask[None, None], scores, -1000000000.0)
        p = _softmax(scores, axis=-1)
        ctx = jnp.einsum('bhqk,bhkd->bhqd', p, v)
        return jnp.einsum('bhqd,hdm->bqm', ctx, w_o)

    def _B_ref(x, mem0, Wq, Wk, Wv, Wo, seg_len):
        B, S, Dm = x.shape
        H, Dh = (Wq.shape[1], Wq.shape[2])
        M = mem0.shape[1]
        scale = Dh ** (-0.5)
        n_seg = S // seg_len
        L = M + seg_len
        idx = jnp.arange(L)
        mask = (idx[:, None] < M) | (idx[:, None] >= idx[None, :])
        mem = mem0
        outs = []
        for s in range(n_seg):
            xs = x[:, s * seg_len:(s + 1) * seg_len, :].copy()
            h = jnp.concatenate([mem, xs], axis=1)
            q = jnp.einsum('btd,dhe->bhte', h, Wq)
            k = jnp.einsum('btd,dhe->bhte', h, Wk)
            v = jnp.einsum('btd,dhe->bhte', h, Wv)
            scores = jnp.einsum('bhqe,bhke->bhqk', q, k) * scale
            scores = jnp.where(mask[None, None], scores, -1000000000.0)
            p = _softmax(scores, axis=-1)
            o = jnp.einsum('bhqk,bhke->bhqe', p, v)
            o = jnp.einsum('bhte,hed->btd', o, Wo)
            mem = o[:, :M, :].copy()
            outs.append(o[:, M:, :])
        return jnp.concatenate(outs, axis=1)
    a = _A_ref(A_x, A_c_kv, A_w_q, A_w_uk, A_w_uv, A_w_o)
    b = _B_ref(B_x, B_mem0, B_Wq, B_Wk, B_Wv, B_Wo, B_seg_len)
    return jnp.concatenate([a, b], axis=-1)
```

```python
import functools

import jax
import jax.numpy as jnp
from jax import lax
import jax.experimental.pallas as pl
import jax.experimental.pallas.tpu as pltpu

F32 = jnp.float32
BF16 = jnp.bfloat16
LOG2E = 1.4426950408889634
NEG = -1e30


def _nn(a, b):
    return jnp.dot(a, b, preferred_element_type=F32)


def _nt(a, b):
    return lax.dot_general(a, b, (((1,), (1,)), ((), ())), preferred_element_type=F32)


def _make_kernel(S, Dm, H, Dh, Dc, M, SEG, BQ=512):
    L = M + SEG
    NSEG = S // SEG
    HD = H * Dh
    qscale = Dh ** -0.5 * LOG2E

    def kernel(axT_hbm, ac_hbm, awq_hbm, awk_hbm, awv_hbm, awoT_hbm,
               bxT_hbm, bmem_hbm, bwq_hbm, bwk_hbm, bwv_hbm, bwoT_hbm,
               out_hbm,
               xTa, xTb, ac, rq, rk, rv, rbq, rbk, rbv, memb,
               ax, awq, awk, awv, awoT, acc,
               bx32, bwq, bwk, bwv, bwoT, obuf, sems):
        def cp(src, dst, i):
            c = pltpu.make_async_copy(src, dst, sems.at[i])
            c.start()
            return c

        c_ax = cp(axT_hbm.at[0], xTa, 0)
        c_ac = cp(ac_hbm.at[0], ac, 1)
        c_aq = cp(awq_hbm, rq, 2)
        c_ak = cp(awk_hbm, rk, 3)
        c_av = cp(awv_hbm, rv, 4)
        c_ao = [cp(awoT_hbm.at[h], awoT.at[:, pl.ds(h * Dh, Dh)], 16 + h) for h in range(H)]
        c_bx = cp(bxT_hbm.at[0], xTb, 5)
        c_bm = cp(bmem_hbm.at[0], memb, 6)
        c_bq = cp(bwq_hbm, rbq, 7)
        c_bk = cp(bwk_hbm, rbk, 8)
        c_bv = cp(bwv_hbm, rbv, 9)
        c_bo = [cp(bwoT_hbm.at[h], bwoT.at[:, pl.ds(h * Dh, Dh)], 16 + H + h) for h in range(H)]

        TC = 256
        c_ax.wait()
        for i in range(S // TC):
            ax[i * TC:(i + 1) * TC, :] = xTa[:, i * TC:(i + 1) * TC].astype(F32).T.astype(BF16)
        c_ac.wait()
        c_aq.wait()
        awq[...] = rq[...].reshape(Dm, HD)
        c_ak.wait()
        awk[...] = rk[...].reshape(Dc, HD)
        c_av.wait()
        awv[...] = rv[...].reshape(Dc, HD)
        for c in c_ao:
            c.wait()
        c_bx.wait()
        for i in range(S // TC):
            bx32[i * TC:(i + 1) * TC, :] = xTb[:, i * TC:(i + 1) * TC].astype(F32).T
        c_bq.wait()
        bwq[...] = rbq[...].reshape(Dm, HD)
        c_bk.wait()
        bwk[...] = rbk[...].reshape(Dm, HD)
        c_bv.wait()
        bwv[...] = rbv[...].reshape(Dm, HD)
        for c in c_bo:
            c.wait()
        c_bm.wait()
        acc[...] = jnp.zeros_like(acc)

        def a_head(h):
            cs = pl.ds(pl.multiple_of(h * Dh, Dh), Dh)
            q = (_nn(ax[...], awq[:, cs]) * qscale).astype(BF16)
            k = _nn(ac[...], awk[:, cs]).astype(BF16)
            v = _nn(ac[...], awv[:, cs]).astype(BF16)
            wo = awoT[:, cs]
            row = lax.broadcasted_iota(jnp.int32, (128, 128), 0)
            col = lax.broadcasted_iota(jnp.int32, (128, 128), 1)
            tri = row >= col
            nsub = BQ // 128
            for i in range(S // BQ):
                qi = q[i * BQ:(i + 1) * BQ]
                pre = _nt(qi, k[0:i * BQ]) if i > 0 else None
                outs = []
                for a in range(nsub):
                    parts = [pre[a * 128:(a + 1) * 128]] if i > 0 else []
                    qa = qi[a * 128:(a + 1) * 128]
                    if a > 0:
                        parts.append(_nt(qa, k[i * BQ:i * BQ + a * 128]))
                    sd = _nt(qa, k[i * BQ + a * 128:i * BQ + (a + 1) * 128])
                    parts.append(jnp.where(tri, sd, NEG))
                    sc = jnp.concatenate(parts, axis=1) if len(parts) > 1 else parts[0]
                    m = jnp.max(sc, axis=1, keepdims=True)
                    p = jnp.exp2(sc - m)
                    l = jnp.sum(p, axis=1, keepdims=True)
                    o = _nn(p.astype(BF16), v[0:i * BQ + (a + 1) * 128])
                    outs.append(o * pltpu.reciprocal(l, approx=True))
                ctx = jnp.concatenate(outs, axis=0).astype(BF16)
                acc[i * BQ:(i + 1) * BQ, :] += _nt(ctx, wo)

        rowb = lax.broadcasted_iota(jnp.int32, (L, L), 0)
        colb = lax.broadcasted_iota(jnp.int32, (L, L), 1)
        maskb = (rowb < M) | (rowb >= colb)

        def b_step(s, mem):
            r0 = pl.multiple_of(s * SEG, SEG)
            hh = jnp.concatenate([mem, bx32[pl.ds(r0, SEG), :]], axis=0)
            q = _nn(hh, bwq[...]) * qscale
            k = _nn(hh, bwk[...]).astype(BF16)
            v = _nn(hh, bwv[...]).astype(BF16)
            outs = []
            for j in range(H):
                hs = slice(j * Dh, (j + 1) * Dh)
                sc = jnp.where(maskb, _nt(q[:, hs], k[:, hs]), NEG)
                m = jnp.max(sc, axis=-1, keepdims=True)
                p = jnp.exp2(sc - m)
                l = jnp.sum(p, axis=-1, keepdims=True)
                a = _nn(p, v[:, hs])
                outs.append(a * pltpu.reciprocal(l, approx=True))
            a = jnp.concatenate(outs, axis=1)
            o = _nt(a, bwoT[...])
            obuf[pl.ds(r0, SEG), Dm:] = o[M:].astype(BF16)
            return o[:M].astype(BF16).astype(F32)

        def body(h, mem):
            a_head(h)
            mem = b_step(2 * h, mem)
            mem = b_step(2 * h + 1, mem)
            return mem

        lax.fori_loop(0, H, body, memb[...].astype(F32))
        obuf[:, :Dm] = acc[...].astype(BF16)
        c = pltpu.make_async_copy(obuf, out_hbm.at[0], sems.at[10])
        c.start()
        c.wait()

    scratch = [
        pltpu.VMEM((Dm, S), BF16), pltpu.VMEM((Dm, S), BF16), pltpu.VMEM((S, Dc), BF16),
        pltpu.VMEM((Dm, H, Dh), BF16), pltpu.VMEM((Dc, H, Dh), BF16), pltpu.VMEM((Dc, H, Dh), BF16),
        pltpu.VMEM((Dm, H, Dh), BF16), pltpu.VMEM((Dm, H, Dh), BF16), pltpu.VMEM((Dm, H, Dh), BF16),
        pltpu.VMEM((M, Dm), BF16),
        pltpu.VMEM((S, Dm), BF16), pltpu.VMEM((Dm, HD), BF16), pltpu.VMEM((Dc, HD), BF16),
        pltpu.VMEM((Dc, HD), BF16), pltpu.VMEM((Dm, HD), BF16), pltpu.VMEM((S, Dm), F32),
        pltpu.VMEM((S, Dm), F32), pltpu.VMEM((Dm, HD), BF16), pltpu.VMEM((Dm, HD), BF16),
        pltpu.VMEM((Dm, HD), BF16), pltpu.VMEM((Dm, HD), BF16), pltpu.VMEM((S, 2 * Dm), BF16),
        pltpu.SemaphoreType.DMA((16 + 2 * H,)),
    ]
    return kernel, scratch


@functools.partial(jax.jit, static_argnames=("B_seg_len",))
def pallas_concat_heads__compressed_kv_cla__memory_aug_recurrent_mem_tr__prompt_kernel(
    A_x, A_c_kv, A_w_q, A_w_uk, A_w_uv, A_w_o,
    B_x, B_mem0, B_Wq, B_Wk, B_Wv, B_Wo, B_seg_len,
):
    B, S, Dm = A_x.shape
    Dc = A_c_kv.shape[-1]
    H, Dh = A_w_q.shape[1], A_w_q.shape[2]
    M = B_mem0.shape[1]
    SEG = int(B_seg_len)
    assert B == 1 and S == 2 * H * SEG
    kernel, scratch = _make_kernel(S, Dm, H, Dh, Dc, M, SEG)
    hbm = pl.BlockSpec(memory_space=pl.ANY)
    return pl.pallas_call(
        kernel,
        out_shape=jax.ShapeDtypeStruct((B, S, 2 * Dm), A_x.dtype),
        in_specs=[hbm] * 12,
        out_specs=hbm,
        scratch_shapes=scratch,
        compiler_params=pltpu.CompilerParams(vmem_limit_bytes=120 * 2 ** 20),
        name="cla_rmt",
    )(
        jnp.swapaxes(A_x, 1, 2), A_c_kv, A_w_q, A_w_uk, A_w_uv, jnp.swapaxes(A_w_o, 1, 2),
        jnp.swapaxes(B_x, 1, 2), B_mem0, B_Wq, B_Wk, B_Wv, jnp.swapaxes(B_Wo, 1, 2),
    )
```

```python
import functools

import jax
import jax.numpy as jnp
from jax import lax
import jax.experimental.pallas as pl
import jax.experimental.pallas.tpu as pltpu

F32 = jnp.float32
BF16 = jnp.bfloat16
U32 = jnp.uint32
LOG2E = 1.4426950408889634
NEG = -1e30


def _nn(a, b):
    return jnp.dot(a, b, preferred_element_type=F32)


def _nt(a, b):
    return lax.dot_general(a, b, (((1,), (1,)), ((), ())), preferred_element_type=F32)


def _half(u, odd):
    bits = (u & jnp.uint32(0xFFFF0000)) if odd else (u << 16)
    return pltpu.bitcast(bits, F32).astype(BF16)


def _drain(*gens):
    for g in gens:
        for _ in g:
            pass


def _make_kernel(S, Dm, H, Dh, Dc, M, SEG, BQ=256, G=4, PC=256, NA=2):
    L = M + SEG
    HD = H * Dh
    NP = H // 2
    NT = 4 * NA
    qscale = Dh ** -0.5 * LOG2E
    KW = (Dm, Dc, Dc)
    KO = (0, Dm, Dm + Dc)

    def kernel(axT_hbm, ac_hbm, awq_hbm, awk_hbm, awv_hbm, awoT_hbm,
               bxT_hbm, bmem_hbm, bwq_hbm, bwk_hbm, bwv_hbm, bwoT_hbm,
               out_hbm,
               xTa, xTb, ac, araw, braw, memb, ax, awq, awk, awv, awoT, ctx,
               bx32, bwq, bwk, bwv, bwoT, bwo, obuf, q0, k0, v0, q1, k1, v1, sems, asem, bsem):
        qs, ks, vs = (q0, q1), (k0, k1), (v0, v1)
        aw32 = [w.bitcast(U32) for w in (awq_hbm, awk_hbm, awv_hbm)]
        bw32 = [w.bitcast(U32) for w in (bwq_hbm, bwk_hbm, bwv_hbm)]

        def a_wcopies(p, b):
            return [pltpu.make_async_copy(aw32[i].at[:, p, :], araw.at[b, pl.ds(KO[i], KW[i]), :], asem.at[b, i])
                    for i in range(3)]

        def cp(src, dst, sem):
            c = pltpu.make_async_copy(src, dst, sem)
            c.start()
            return c

        c_ax = cp(axT_hbm.at[0], xTa, sems.at[0])
        c_ac = cp(ac_hbm.at[0], ac, sems.at[1])
        for p in range(2):
            for c in a_wcopies(p, p):
                c.start()
        TC = 256
        c_ax.wait()
        for i in range(S // TC):
            ax[i * TC:(i + 1) * TC, :] = xTa[:, i * TC:(i + 1) * TC].astype(F32).T.astype(BF16)
        c_ac.wait()
        for c in a_wcopies(0, 0):
            c.wait()
        c_bw = [[cp(bw32[i].at[:, p, :], braw.at[i, p], bsem.at[i * NP + p]) for p in range(NP)] for i in range(3)]
        c_bx = cp(bxT_hbm.at[0], xTb, sems.at[2])
        c_bm = cp(bmem_hbm.at[0], memb, sems.at[3])
        c_bo = [cp(bwoT_hbm.at[h], bwoT.at[:, pl.ds(h * Dh, Dh)], bsem.at[3 * NP + h]) for h in range(H)]

        def a_proj(b, odd, slot):
            awq[...] = _half(araw[b, KO[0]:KO[0] + KW[0], :], odd)
            awk[...] = _half(araw[b, KO[1]:KO[1] + KW[1], :], odd)
            awv[...] = _half(araw[b, KO[2]:KO[2] + KW[2], :], odd)
            for r in range(S // PC):
                rs = slice(r * PC, (r + 1) * PC)
                qs[slot][rs, :] = (_nn(ax[rs, :], awq[...]) * qscale).astype(BF16)
                yield PC * 5 // 4
                ks[slot][rs, :] = _nn(ac[rs, :], awk[...]).astype(BF16)
                yield PC
                vs[slot][rs, :] = _nn(ac[rs, :], awv[...]).astype(BF16)
                yield PC

        def a_attn(h, slot):
            cs = pl.ds(pl.multiple_of(h * Dh, Dh), Dh)
            row = lax.broadcasted_iota(jnp.int32, (128, 128), 0)
            col = lax.broadcasted_iota(jnp.int32, (128, 128), 1)
            tri = row >= col
            nsub = BQ // 128

            def scores(i):
                qi = qs[slot][i * BQ:(i + 1) * BQ, :]
                pre = _nt(qi, ks[slot][0:i * BQ, :]) if i > 0 else None
                res = []
                for a in range(nsub):
                    parts = [pre[a * 128:(a + 1) * 128]] if i > 0 else []
                    qa = qi[a * 128:(a + 1) * 128]
                    if a > 0:
                        parts.append(_nt(qa, ks[slot][i * BQ:i * BQ + a * 128, :]))
                    sd = _nt(qa, ks[slot][i * BQ + a * 128:i * BQ + (a + 1) * 128, :])
                    parts.append(jnp.where(tri, sd, NEG))
                    res.append(jnp.concatenate(parts, axis=1) if len(parts) > 1 else parts[0])
                return res

            nb = S // BQ
            cur = scores(0)
            yield 32 * nsub * (nsub + 1) // 2
            for i in range(nb):
                nxt = None
                if i + 1 < nb:
                    nxt = scores(i + 1)
                    yield BQ * (i + 1) * nsub // 4 + 32 * nsub * (nsub + 1) // 2
                for a in range(nsub):
                    sc = cur[a]
                    m = jnp.max(sc, axis=1, keepdims=True)
                    p = jnp.exp2(sc - m)
                    l = jnp.sum(p, axis=1, keepdims=True)
                    o = _nn(p.astype(BF16), vs[slot][0:i * BQ + (a + 1) * 128, :])
                    r0 = i * BQ + a * 128
                    ctx[r0:r0 + 128, cs] = (o * pltpu.reciprocal(l, approx=True)).astype(BF16)
                    yield 32 * (i * nsub + a + 1)
                cur = nxt

        rowb = lax.broadcasted_iota(jnp.int32, (L, L), 0)
        colb = lax.broadcasted_iota(jnp.int32, (L, L), 1)
        maskb = (rowb < M) | (rowb >= colb)
        NG = H // G
        GW = G * Dh

        def b_steps(s0, n, state):
            for s in range(n):
                r0 = pl.multiple_of((s0 + s) * SEG, SEG)
                hh = jnp.concatenate([state[0], bx32[pl.ds(r0, SEG), :]], axis=0)
                qkv = []
                for g in range(NG):
                    cs = slice(g * GW, (g + 1) * GW)
                    q = _nn(hh, bwq[:, cs]) * qscale
                    k = _nn(hh, bwk[:, cs]).astype(BF16)
                    v = _nn(hh, bwv[:, cs]).astype(BF16)
                    qkv.append((q, k, v))
                    yield 3 * 5 * G * L // 4
                scs = []
                for g in range(NG):
                    q, k, v = qkv[g]
                    for j in range(G):
                        hs = slice(j * Dh, (j + 1) * Dh)
                        scs.append(jnp.where(maskb, _nt(q[:, hs], k[:, hs]), NEG))
                yield None
                ps = []
                for sc in scs:
                    m = jnp.max(sc, axis=-1, keepdims=True)
                    p = jnp.exp2(sc - m)
                    l = jnp.sum(p, axis=-1, keepdims=True)
                    ps.append((p, pltpu.reciprocal(l, approx=True)))
                yield None
                att = []
                for g in range(NG):
                    v = qkv[g][2]
                    outs = [_nn(ps[g * G + j][0], v[:, j * Dh:(j + 1) * Dh]) * ps[g * G + j][1] for j in range(G)]
                    att.append(jnp.concatenate(outs, axis=1) if G > 1 else outs[0])
                yield None
                o = None
                for g in range(NG):
                    t = _nn(att[g], bwo[g * GW:(g + 1) * GW, :])
                    o = t if o is None else o + t
                    yield 5 * G * L // 4
                obuf[pl.ds(r0, SEG), Dm:] = o[M:].astype(BF16)
                state[0] = o[:M].astype(BF16).astype(F32)

        def interleave(ga, gp, gb, ta, tb, nfill):
            da = db = 0.0
            a_alive = True
            for c in gb:
                if c is None:
                    for _ in range(nfill):
                        next(gp, None)
                    continue
                db += c
                while a_alive and da / ta < db / tb:
                    ca = next(ga, None)
                    if ca is None:
                        a_alive = False
                    else:
                        da += ca
            _drain(ga, gp)

        def a_pair(hp, gb_for_slot):
            @pl.when(hp + 2 < NP)
            def _():
                for c in a_wcopies(hp + 2, (hp + 2) % 3):
                    c.start()
            for slot in range(2):
                if slot == 1:
                    @pl.when(hp + 1 < NP)
                    def _():
                        for c in a_wcopies(hp + 1, (hp + 1) % 3):
                            c.wait()
                nb = hp if slot == 0 else jnp.minimum(hp + 1, NP - 1)
                gb_for_slot(slot, a_attn(2 * hp + slot, slot), a_proj(nb % 3, slot == 0, 1 - slot))

        _drain(a_proj(0, False, 0))

        def body_a(hp, carry):
            def run(slot, ga, gp):
                interleave(ga, iter(()), gp, 8704.0, 6656.0, 0)
            a_pair(hp, run)
            return carry

        lax.fori_loop(0, NA, body_a, 0)

        for i, dst in enumerate((bwq, bwk, bwv)):
            for p in range(NP):
                c_bw[i][p].wait()
                u = braw[i, p]
                dst[:, (2 * p) * Dh:(2 * p + 1) * Dh] = _half(u, False)
                dst[:, (2 * p + 1) * Dh:(2 * p + 2) * Dh] = _half(u, True)
        c_bx.wait()
        for i in range(S // TC):
            bx32[i * TC:(i + 1) * TC, :] = xTb[:, i * TC:(i + 1) * TC].astype(F32).T
        for c in c_bo:
            c.wait()
        for h in range(H):
            bwo[h * Dh:(h + 1) * Dh, :] = bwoT[:, h * Dh:(h + 1) * Dh].astype(F32).T.astype(BF16)
        c_bm.wait()
        c_ao = [cp(awoT_hbm.at[h], awoT.at[:, pl.ds(h * Dh, Dh)], bsem.at[3 * NP + H + h]) for h in range(H)]

        def body(hp, mem):
            state = [mem]

            def run(slot, ga, gp):
                interleave(ga, gp, b_steps(4 * (hp - NA) + 2 * slot, 2, state), 8704.0, 12800.0, 3 * (S // PC) // 6)
            a_pair(hp, run)
            return state[0]

        mem = lax.fori_loop(NA, NP, body, memb[...].astype(F32))
        for c in c_ao:
            c.wait()
        RT = S // NT

        def a_out(t):
            for j in range(RT // 32):
                rs = pl.ds(pl.multiple_of(t * RT + j * 32, 32), 32)
                yield rs

        def body_t(t, mem):
            state = [mem]

            def oproj():
                r0 = pl.multiple_of(t * RT, RT)
                accs = None
                for g in range(8):
                    cs = slice(g * HD // 8, (g + 1) * HD // 8)
                    tt = _nt(ctx[pl.ds(r0, RT), cs], awoT[:, cs])
                    accs = tt if accs is None else accs + tt
                    yield RT * 5
                obuf[pl.ds(r0, RT), :Dm] = accs.astype(BF16)

            g = oproj()
            gb = b_steps(S // SEG - NT + t, 1, state)
            n = 0
            for c in gb:
                n += 1
                if c is None or n % 3 == 0:
                    next(g, None)
            _drain(g)
            return state[0]

        lax.fori_loop(0, NT, body_t, mem)
        c = pltpu.make_async_copy(obuf, out_hbm.at[0], sems.at[4])
        c.start()
        c.wait()

    scratch = [
        pltpu.VMEM((Dm, S), BF16), pltpu.VMEM((Dm, S), BF16), pltpu.VMEM((S, Dc), BF16),
        pltpu.VMEM((3, Dm + 2 * Dc, Dh), U32), pltpu.VMEM((3, NP, Dm, Dh), U32), pltpu.VMEM((M, Dm), BF16),
        pltpu.VMEM((S, Dm), BF16), pltpu.VMEM((Dm, Dh), BF16), pltpu.VMEM((Dc, Dh), BF16),
        pltpu.VMEM((Dc, Dh), BF16), pltpu.VMEM((Dm, HD), BF16), pltpu.VMEM((S, HD), BF16),
        pltpu.VMEM((S, Dm), F32), pltpu.VMEM((Dm, HD), BF16), pltpu.VMEM((Dm, HD), BF16),
        pltpu.VMEM((Dm, HD), BF16), pltpu.VMEM((Dm, HD), BF16), pltpu.VMEM((HD, Dm), BF16),
        pltpu.VMEM((S, 2 * Dm), BF16),
        *[pltpu.VMEM((S, Dh), BF16) for _ in range(6)],
        pltpu.SemaphoreType.DMA((8,)), pltpu.SemaphoreType.DMA((3, 3)),
        pltpu.SemaphoreType.DMA((3 * NP + 2 * H,)),
    ]
    return kernel, scratch


@functools.partial(jax.jit, static_argnames=("B_seg_len",))
def pallas_concat_heads__compressed_kv_cla__memory_aug_recurrent_mem_tr__prompt_kernel(
    A_x, A_c_kv, A_w_q, A_w_uk, A_w_uv, A_w_o,
    B_x, B_mem0, B_Wq, B_Wk, B_Wv, B_Wo, B_seg_len,
):
    B, S, Dm = A_x.shape
    Dc = A_c_kv.shape[-1]
    H, Dh = A_w_q.shape[1], A_w_q.shape[2]
    M = B_mem0.shape[1]
    SEG = int(B_seg_len)
    assert B == 1 and S == 2 * H * SEG
    kernel, scratch = _make_kernel(S, Dm, H, Dh, Dc, M, SEG)
    hbm = pl.BlockSpec(memory_space=pl.ANY)
    return pl.pallas_call(
        kernel,
        out_shape=jax.ShapeDtypeStruct((B, S, 2 * Dm), A_x.dtype),
        in_specs=[hbm] * 12,
        out_specs=hbm,
        scratch_shapes=scratch,
        compiler_params=pltpu.CompilerParams(vmem_limit_bytes=124 * 2 ** 20),
        name="cla_rmt",
    )(
        jnp.swapaxes(A_x, 1, 2), A_c_kv, A_w_q, A_w_uk, A_w_uv, jnp.swapaxes(A_w_o, 1, 2),
        jnp.swapaxes(B_x, 1, 2), B_mem0, B_Wq, B_Wk, B_Wv, jnp.swapaxes(B_Wo, 1, 2),
    )
```

```python
import functools

import jax
import jax.numpy as jnp
from jax import lax
import jax.experimental.pallas as pl
import jax.experimental.pallas.tpu as pltpu

F32 = jnp.float32
BF16 = jnp.bfloat16
U32 = jnp.uint32
LOG2E = 1.4426950408889634
NEG = -1e30


def _nn(a, b):
    return jnp.dot(a, b, preferred_element_type=F32)


def _nt(a, b):
    return lax.dot_general(a, b, (((1,), (1,)), ((), ())), preferred_element_type=F32)


def _half(u, odd):
    if isinstance(odd, bool):
        bits = (u & jnp.uint32(0xFFFF0000)) if odd else (u << 16)
    else:
        bits = jnp.where(odd, u, u << 16) & jnp.uint32(0xFFFF0000)
    return pltpu.bitcast(bits, F32).astype(BF16)


def _drain(*gens):
    for g in gens:
        for _ in g:
            pass


def _make_kernel(S, Dm, H, Dh, Dc, M, SEG, BQ=256, G=4, PC=256, NA=2):
    L = M + SEG
    HD = H * Dh
    NP = H // 2
    NT = 4 * NA
    qscale = Dh ** -0.5 * LOG2E
    KW = (Dm, Dc, Dc)
    KO = (0, Dm, Dm + Dc)

    def kernel(axT_hbm, ac_hbm, awq_hbm, awk_hbm, awv_hbm, awoT_hbm,
               bxT_hbm, bmem_hbm, bwq_hbm, bwk_hbm, bwv_hbm, bwoT_hbm,
               out_hbm,
               xTa, xTb, ac, araw, braw, memb, ax, awq, awk, awv, awoT, ctx,
               bx32, bwq, bwk, bwv, bwoT, bwo, obuf, qs, ks, vs, sems, asem, bsem):
        aw32 = [w.bitcast(U32) for w in (awq_hbm, awk_hbm, awv_hbm)]
        bw32 = [w.bitcast(U32) for w in (bwq_hbm, bwk_hbm, bwv_hbm)]

        def a_wcopies(p, b):
            return [pltpu.make_async_copy(aw32[i].at[:, p, :], araw.at[b, pl.ds(KO[i], KW[i]), :], asem.at[b, i])
                    for i in range(3)]

        def cp(src, dst, sem):
            c = pltpu.make_async_copy(src, dst, sem)
            c.start()
            return c

        c_ax = cp(axT_hbm.at[0], xTa, sems.at[0])
        c_ac = cp(ac_hbm.at[0], ac, sems.at[1])
        for p in range(2):
            for c in a_wcopies(p, p):
                c.start()
        TC = 256
        c_ax.wait()
        for i in range(S // TC):
            ax[i * TC:(i + 1) * TC, :] = xTa[:, i * TC:(i + 1) * TC].astype(F32).T.astype(BF16)
        c_ac.wait()
        for c in a_wcopies(0, 0):
            c.wait()
        c_bw = [[cp(bw32[i].at[:, p, :], braw.at[i, p], bsem.at[i * NP + p]) for p in range(NP)] for i in range(3)]
        c_bx = cp(bxT_hbm.at[0], xTb, sems.at[2])
        c_bm = cp(bmem_hbm.at[0], memb, sems.at[3])
        c_bo = [cp(bwoT_hbm.at[h], bwoT.at[:, pl.ds(h * Dh, Dh)], bsem.at[3 * NP + h]) for h in range(H)]

        def a_proj(b, odd, slot):
            awq[...] = _half(araw[b, KO[0]:KO[0] + KW[0], :], odd)
            awk[...] = _half(araw[b, KO[1]:KO[1] + KW[1], :], odd)
            awv[...] = _half(araw[b, KO[2]:KO[2] + KW[2], :], odd)
            for r in range(S // PC):
                rs = slice(r * PC, (r + 1) * PC)
                qs[slot, rs, :] = (_nn(ax[rs, :], awq[...]) * qscale).astype(BF16)
                yield PC * 5 // 4
                ks[slot, rs, :] = _nn(ac[rs, :], awk[...]).astype(BF16)
                yield PC
                vs[slot, rs, :] = _nn(ac[rs, :], awv[...]).astype(BF16)
                yield PC

        def a_attn(h, slot):
            cs = pl.ds(pl.multiple_of(h * Dh, Dh), Dh)
            row = lax.broadcasted_iota(jnp.int32, (128, 128), 0)
            col = lax.broadcasted_iota(jnp.int32, (128, 128), 1)
            tri = row >= col
            nsub = BQ // 128

            def scores(i):
                qi = qs[slot, i * BQ:(i + 1) * BQ, :]
                pre = _nt(qi, ks[slot, 0:i * BQ, :]) if i > 0 else None
                res = []
                for a in range(nsub):
                    parts = [pre[a * 128:(a + 1) * 128]] if i > 0 else []
                    qa = qi[a * 128:(a + 1) * 128]
                    if a > 0:
                        parts.append(_nt(qa, ks[slot, i * BQ:i * BQ + a * 128, :]))
                    sd = _nt(qa, ks[slot, i * BQ + a * 128:i * BQ + (a + 1) * 128, :])
                    parts.append(jnp.where(tri, sd, NEG))
                    res.append(jnp.concatenate(parts, axis=1) if len(parts) > 1 else parts[0])
                return res

            nb = S // BQ
            cur = scores(0)
            yield 32 * nsub * (nsub + 1) // 2
            for i in range(nb):
                nxt = None
                if i + 1 < nb:
                    nxt = scores(i + 1)
                    yield BQ * (i + 1) * nsub // 4 + 32 * nsub * (nsub + 1) // 2
                for a in range(nsub):
                    sc = cur[a]
                    m = jnp.max(sc, axis=1, keepdims=True)
                    p = jnp.exp2(sc - m)
                    l = jnp.sum(p, axis=1, keepdims=True)
                    o = _nn(p.astype(BF16), vs[slot, 0:i * BQ + (a + 1) * 128, :])
                    r0 = i * BQ + a * 128
                    ctx[r0:r0 + 128, cs] = (o * pltpu.reciprocal(l, approx=True)).astype(BF16)
                    yield 32 * (i * nsub + a + 1)
                cur = nxt

        rowb = lax.broadcasted_iota(jnp.int32, (L, L), 0)
        colb = lax.broadcasted_iota(jnp.int32, (L, L), 1)
        maskb = (rowb < M) | (rowb >= colb)
        NG = H // G
        GW = G * Dh

        def b_steps(s0, n, state):
            for s in range(n):
                r0 = pl.multiple_of((s0 + s) * SEG, SEG)
                hh = jnp.concatenate([state[0], bx32[pl.ds(r0, SEG), :]], axis=0)
                qkv = []
                for g in range(NG):
                    cs = slice(g * GW, (g + 1) * GW)
                    q = _nn(hh, bwq[:, cs]) * qscale
                    k = _nn(hh, bwk[:, cs]).astype(BF16)
                    v = _nn(hh, bwv[:, cs]).astype(BF16)
                    qkv.append((q, k, v))
                    yield 3 * 5 * G * L // 4
                scs = []
                for g in range(NG):
                    q, k, v = qkv[g]
                    for j in range(G):
                        hs = slice(j * Dh, (j + 1) * Dh)
                        scs.append(jnp.where(maskb, _nt(q[:, hs], k[:, hs]), NEG))
                yield None
                ps = []
                for sc in scs:
                    m = jnp.max(sc, axis=-1, keepdims=True)
                    p = jnp.exp2(sc - m)
                    l = jnp.sum(p, axis=-1, keepdims=True)
                    ps.append((p, pltpu.reciprocal(l, approx=True)))
                yield None
                att = []
                for g in range(NG):
                    v = qkv[g][2]
                    outs = [_nn(ps[g * G + j][0], v[:, j * Dh:(j + 1) * Dh]) * ps[g * G + j][1] for j in range(G)]
                    att.append(jnp.concatenate(outs, axis=1) if G > 1 else outs[0])
                yield None
                o = None
                for g in range(NG):
                    t = _nn(att[g], bwo[g * GW:(g + 1) * GW, :])
                    o = t if o is None else o + t
                    yield 5 * G * L // 4
                obuf[pl.ds(r0, SEG), Dm:] = o[M:].astype(BF16)
                state[0] = o[:M].astype(BF16).astype(F32)

        def interleave(ga, gp, gb, ta, tb, nfill):
            da = db = 0.0
            a_alive = True
            for c in gb:
                if c is None:
                    for _ in range(nfill):
                        next(gp, None)
                    continue
                db += c
                while a_alive and da / ta < db / tb:
                    ca = next(ga, None)
                    if ca is None:
                        a_alive = False
                    else:
                        da += ca
            _drain(ga, gp)

        def a_streams(h):
            @pl.when((h % 2 == 0) & (h // 2 + 2 < NP))
            def _():
                for c in a_wcopies(h // 2 + 2, (h // 2 + 2) % 3):
                    c.start()

            @pl.when((h % 2 == 1) & ((h + 1) // 2 < NP))
            def _():
                for c in a_wcopies((h + 1) // 2, ((h + 1) // 2) % 3):
                    c.wait()
            hn = jnp.minimum(h + 1, H - 1)
            return a_attn(h, h % 2), a_proj((hn // 2) % 3, hn % 2 == 1, (h + 1) % 2)

        _drain(a_proj(0, False, 0))

        def body_a(h, carry):
            ga, gp = a_streams(h)
            interleave(ga, iter(()), gp, 8704.0, 6656.0, 0)
            return carry

        lax.fori_loop(0, 2 * NA, body_a, 0)

        for i, dst in enumerate((bwq, bwk, bwv)):
            for p in range(NP):
                c_bw[i][p].wait()
                u = braw[i, p]
                dst[:, (2 * p) * Dh:(2 * p + 1) * Dh] = _half(u, False)
                dst[:, (2 * p + 1) * Dh:(2 * p + 2) * Dh] = _half(u, True)
        c_bx.wait()
        for i in range(S // TC):
            bx32[i * TC:(i + 1) * TC, :] = xTb[:, i * TC:(i + 1) * TC].astype(F32).T
        for c in c_bo:
            c.wait()
        for h in range(H):
            bwo[h * Dh:(h + 1) * Dh, :] = bwoT[:, h * Dh:(h + 1) * Dh].astype(F32).T.astype(BF16)
        c_bm.wait()
        c_ao = [cp(awoT_hbm.at[h], awoT.at[:, pl.ds(h * Dh, Dh)], bsem.at[3 * NP + H + h]) for h in range(H)]

        def body(h, mem):
            state = [mem]
            ga, gp = a_streams(h)
            interleave(ga, gp, b_steps(2 * (h - 2 * NA), 2, state), 8704.0, 12800.0, 3 * (S // PC) // 6)
            return state[0]

        mem = lax.fori_loop(2 * NA, H, body, memb[...].astype(F32))
        for c in c_ao:
            c.wait()
        RT = S // NT

        def a_out(t):
            for j in range(RT // 32):
                rs = pl.ds(pl.multiple_of(t * RT + j * 32, 32), 32)
                yield rs

        def body_t(t, mem):
            state = [mem]

            def oproj():
                r0 = pl.multiple_of(t * RT, RT)
                accs = None
                for g in range(8):
                    cs = slice(g * HD // 8, (g + 1) * HD // 8)
                    tt = _nt(ctx[pl.ds(r0, RT), cs], awoT[:, cs])
                    accs = tt if accs is None else accs + tt
                    yield RT * 5
                obuf[pl.ds(r0, RT), :Dm] = accs.astype(BF16)

            g = oproj()
            gb = b_steps(S // SEG - NT + t, 1, state)
            n = 0
            for c in gb:
                n += 1
                if c is None or n % 3 == 0:
                    next(g, None)
            _drain(g)
            return state[0]

        lax.fori_loop(0, NT, body_t, mem)
        c = pltpu.make_async_copy(obuf, out_hbm.at[0], sems.at[4])
        c.start()
        c.wait()

    scratch = [
        pltpu.VMEM((Dm, S), BF16), pltpu.VMEM((Dm, S), BF16), pltpu.VMEM((S, Dc), BF16),
        pltpu.VMEM((3, Dm + 2 * Dc, Dh), U32), pltpu.VMEM((3, NP, Dm, Dh), U32), pltpu.VMEM((M, Dm), BF16),
        pltpu.VMEM((S, Dm), BF16), pltpu.VMEM((Dm, Dh), BF16), pltpu.VMEM((Dc, Dh), BF16),
        pltpu.VMEM((Dc, Dh), BF16), pltpu.VMEM((Dm, HD), BF16), pltpu.VMEM((S, HD), BF16),
        pltpu.VMEM((S, Dm), F32), pltpu.VMEM((Dm, HD), BF16), pltpu.VMEM((Dm, HD), BF16),
        pltpu.VMEM((Dm, HD), BF16), pltpu.VMEM((Dm, HD), BF16), pltpu.VMEM((HD, Dm), BF16),
        pltpu.VMEM((S, 2 * Dm), BF16),
        *[pltpu.VMEM((2, S, Dh), BF16) for _ in range(3)],
        pltpu.SemaphoreType.DMA((8,)), pltpu.SemaphoreType.DMA((3, 3)),
        pltpu.SemaphoreType.DMA((3 * NP + 2 * H,)),
    ]
    return kernel, scratch


@functools.partial(jax.jit, static_argnames=("B_seg_len",))
def pallas_concat_heads__compressed_kv_cla__memory_aug_recurrent_mem_tr__prompt_kernel(
    A_x, A_c_kv, A_w_q, A_w_uk, A_w_uv, A_w_o,
    B_x, B_mem0, B_Wq, B_Wk, B_Wv, B_Wo, B_seg_len,
):
    B, S, Dm = A_x.shape
    Dc = A_c_kv.shape[-1]
    H, Dh = A_w_q.shape[1], A_w_q.shape[2]
    M = B_mem0.shape[1]
    SEG = int(B_seg_len)
    assert B == 1 and S == 2 * H * SEG
    kernel, scratch = _make_kernel(S, Dm, H, Dh, Dc, M, SEG)
    hbm = pl.BlockSpec(memory_space=pl.ANY)
    return pl.pallas_call(
        kernel,
        out_shape=jax.ShapeDtypeStruct((B, S, 2 * Dm), A_x.dtype),
        in_specs=[hbm] * 12,
        out_specs=hbm,
        scratch_shapes=scratch,
        compiler_params=pltpu.CompilerParams(vmem_limit_bytes=124 * 2 ** 20),
        name="cla_rmt",
    )(
        jnp.swapaxes(A_x, 1, 2), A_c_kv, A_w_q, A_w_uk, A_w_uv, jnp.swapaxes(A_w_o, 1, 2),
        jnp.swapaxes(B_x, 1, 2), B_mem0, B_Wq, B_Wk, B_Wv, jnp.swapaxes(B_Wo, 1, 2),
    )
```

```python
import functools

import jax
import jax.numpy as jnp
from jax import lax
import jax.experimental.pallas as pl
import jax.experimental.pallas.tpu as pltpu

F32 = jnp.float32
BF16 = jnp.bfloat16
U32 = jnp.uint32
LOG2E = 1.4426950408889634
NEG = -1e30


def _nn(a, b):
    return jnp.dot(a, b, preferred_element_type=F32)


def _nt(a, b):
    return lax.dot_general(a, b, (((1,), (1,)), ((), ())), preferred_element_type=F32)


def _half(u, odd):
    if isinstance(odd, bool):
        bits = (u & jnp.uint32(0xFFFF0000)) if odd else (u << 16)
    else:
        bits = jnp.where(odd, u, u << 16) & jnp.uint32(0xFFFF0000)
    return pltpu.bitcast(bits, F32).astype(BF16)


def _drain(*gens):
    for g in gens:
        for _ in g:
            pass


def _make_kernel(S, Dm, H, Dh, Dc, M, SEG, BQ=256, G=4, PC=256, NA=2):
    L = M + SEG
    HD = H * Dh
    NP = H // 2
    NT = 4 * NA
    assert (NT - 1) * (S // NT) <= S - NT * SEG
    qscale = Dh ** -0.5 * LOG2E
    KW = (Dm, Dc, Dc)
    KO = (0, Dm, Dm + Dc)

    def kernel(axT_hbm, ac_hbm, awq_hbm, awk_hbm, awv_hbm, awoT_hbm,
               bxT_hbm, bmem_hbm, bwq_hbm, bwk_hbm, bwv_hbm, bwoT_hbm,
               out_hbm,
               xTa, xTb, ac, araw, braw, memb, ax, awq, awk, awv, awoT, ctx,
               bx32, bwq, bwk, bwv, bwoT, bwo, obuf, qs, ks, vs, sems, asem, bsem, osem):
        aw32 = [w.bitcast(U32) for w in (awq_hbm, awk_hbm, awv_hbm)]
        bw32 = [w.bitcast(U32) for w in (bwq_hbm, bwk_hbm, bwv_hbm)]

        def a_wcopies(p, b):
            return [pltpu.make_async_copy(aw32[i].at[:, p, :], araw.at[b, pl.ds(KO[i], KW[i]), :], asem.at[b, i])
                    for i in range(3)]

        def cp(src, dst, sem):
            c = pltpu.make_async_copy(src, dst, sem)
            c.start()
            return c

        c_ax = cp(axT_hbm.at[0], xTa, sems.at[0])
        c_ac = cp(ac_hbm.at[0], ac, sems.at[1])
        for p in range(2):
            for c in a_wcopies(p, p):
                c.start()
        TC = 256
        c_ax.wait()
        for i in range(S // TC):
            ax[i * TC:(i + 1) * TC, :] = xTa[:, i * TC:(i + 1) * TC].astype(F32).T.astype(BF16)
        c_ac.wait()
        for c in a_wcopies(0, 0):
            c.wait()
        c_bw = [[cp(bw32[i].at[:, p, :], braw.at[i, p], bsem.at[i * NP + p]) for p in range(NP)] for i in range(3)]
        c_bx = cp(bxT_hbm.at[0], xTb, sems.at[2])
        c_bm = cp(bmem_hbm.at[0], memb, sems.at[3])
        c_bo = [cp(bwoT_hbm.at[h], bwoT.at[:, pl.ds(h * Dh, Dh)], bsem.at[3 * NP + h]) for h in range(H)]

        def a_proj(b, odd, slot):
            awq[...] = _half(araw[b, KO[0]:KO[0] + KW[0], :], odd)
            awk[...] = _half(araw[b, KO[1]:KO[1] + KW[1], :], odd)
            awv[...] = _half(araw[b, KO[2]:KO[2] + KW[2], :], odd)
            for r in range(S // PC):
                rs = slice(r * PC, (r + 1) * PC)
                qs[slot, rs, :] = (_nn(ax[rs, :], awq[...]) * qscale).astype(BF16)
                yield PC * 5 // 4
                ks[slot, rs, :] = _nn(ac[rs, :], awk[...]).astype(BF16)
                yield PC
                vs[slot, rs, :] = _nn(ac[rs, :], awv[...]).astype(BF16)
                yield PC

        def a_attn(h, slot):
            cs = pl.ds(pl.multiple_of(h * Dh, Dh), Dh)
            row = lax.broadcasted_iota(jnp.int32, (128, 128), 0)
            col = lax.broadcasted_iota(jnp.int32, (128, 128), 1)
            tri = row >= col
            nsub = BQ // 128

            def scores(i):
                qi = qs[slot, i * BQ:(i + 1) * BQ, :]
                pre = _nt(qi, ks[slot, 0:i * BQ, :]) if i > 0 else None
                res = []
                for a in range(nsub):
                    parts = [pre[a * 128:(a + 1) * 128]] if i > 0 else []
                    qa = qi[a * 128:(a + 1) * 128]
                    if a > 0:
                        parts.append(_nt(qa, ks[slot, i * BQ:i * BQ + a * 128, :]))
                    sd = _nt(qa, ks[slot, i * BQ + a * 128:i * BQ + (a + 1) * 128, :])
                    parts.append(jnp.where(tri, sd, NEG))
                    res.append(jnp.concatenate(parts, axis=1) if len(parts) > 1 else parts[0])
                return res

            nb = S // BQ
            cur = scores(0)
            yield 32 * nsub * (nsub + 1) // 2
            for i in range(nb):
                nxt = None
                if i + 1 < nb:
                    nxt = scores(i + 1)
                    yield BQ * (i + 1) * nsub // 4 + 32 * nsub * (nsub + 1) // 2
                for a in range(nsub):
                    sc = cur[a]
                    m = jnp.max(sc, axis=1, keepdims=True)
                    p = jnp.exp2(sc - m)
                    l = jnp.sum(p, axis=1, keepdims=True)
                    o = _nn(p.astype(BF16), vs[slot, 0:i * BQ + (a + 1) * 128, :])
                    r0 = i * BQ + a * 128
                    ctx[r0:r0 + 128, cs] = (o * pltpu.reciprocal(l, approx=True)).astype(BF16)
                    yield 32 * (i * nsub + a + 1)
                cur = nxt

        rowb = lax.broadcasted_iota(jnp.int32, (L, L), 0)
        colb = lax.broadcasted_iota(jnp.int32, (L, L), 1)
        maskb = (rowb < M) | (rowb >= colb)
        NG = H // G
        GW = G * Dh

        def b_steps(s0, n, state):
            for s in range(n):
                r0 = pl.multiple_of((s0 + s) * SEG, SEG)
                hh = jnp.concatenate([state[0], bx32[pl.ds(r0, SEG), :]], axis=0)
                qkv = []
                for g in range(NG):
                    cs = slice(g * GW, (g + 1) * GW)
                    q = _nn(hh, bwq[:, cs]) * qscale
                    k = _nn(hh, bwk[:, cs]).astype(BF16)
                    v = _nn(hh, bwv[:, cs]).astype(BF16)
                    qkv.append((q, k, v))
                    yield 3 * 5 * G * L // 4
                scs = []
                for g in range(NG):
                    q, k, v = qkv[g]
                    for j in range(G):
                        hs = slice(j * Dh, (j + 1) * Dh)
                        scs.append(jnp.where(maskb, _nt(q[:, hs], k[:, hs]), NEG))
                yield None
                ps = []
                for sc in scs:
                    m = jnp.max(sc, axis=-1, keepdims=True)
                    p = jnp.exp2(sc - m)
                    l = jnp.sum(p, axis=-1, keepdims=True)
                    ps.append((p, pltpu.reciprocal(l, approx=True)))
                yield None
                att = []
                for g in range(NG):
                    v = qkv[g][2]
                    outs = [_nn(ps[g * G + j][0], v[:, j * Dh:(j + 1) * Dh]) * ps[g * G + j][1] for j in range(G)]
                    att.append(jnp.concatenate(outs, axis=1) if G > 1 else outs[0])
                yield None
                o = None
                for g in range(NG):
                    t = _nn(att[g], bwo[g * GW:(g + 1) * GW, :])
                    o = t if o is None else o + t
                    yield 5 * G * L // 4
                obuf[pl.ds(r0, SEG), Dm:] = o[M:].astype(BF16)
                state[0] = o[:M].astype(BF16).astype(F32)

        def interleave(ga, gp, gb, ta, tb, nfill):
            da = db = 0.0
            a_alive = True
            for c in gb:
                if c is None:
                    for _ in range(nfill):
                        next(gp, None)
                    continue
                db += c
                while a_alive and da / ta < db / tb:
                    ca = next(ga, None)
                    if ca is None:
                        a_alive = False
                    else:
                        da += ca
            _drain(ga, gp)

        def a_streams(h):
            @pl.when((h % 2 == 0) & (h // 2 + 2 < NP))
            def _():
                for c in a_wcopies(h // 2 + 2, (h // 2 + 2) % 3):
                    c.start()

            @pl.when((h % 2 == 1) & ((h + 1) // 2 < NP))
            def _():
                for c in a_wcopies((h + 1) // 2, ((h + 1) // 2) % 3):
                    c.wait()
            hn = jnp.minimum(h + 1, H - 1)
            return a_attn(h, h % 2), a_proj((hn // 2) % 3, hn % 2 == 1, (h + 1) % 2)

        _drain(a_proj(0, False, 0))

        def body_a(h, carry):
            ga, gp = a_streams(h)
            interleave(ga, iter(()), gp, 8704.0, 6656.0, 0)
            return carry

        lax.fori_loop(0, 2 * NA, body_a, 0)

        for i, dst in enumerate((bwq, bwk, bwv)):
            for p in range(NP):
                c_bw[i][p].wait()
                u = braw[i, p]
                dst[:, (2 * p) * Dh:(2 * p + 1) * Dh] = _half(u, False)
                dst[:, (2 * p + 1) * Dh:(2 * p + 2) * Dh] = _half(u, True)
        c_bx.wait()
        for i in range(S // TC):
            bx32[i * TC:(i + 1) * TC, :] = xTb[:, i * TC:(i + 1) * TC].astype(F32).T
        for c in c_bo:
            c.wait()
        for h in range(H):
            bwo[h * Dh:(h + 1) * Dh, :] = bwoT[:, h * Dh:(h + 1) * Dh].astype(F32).T.astype(BF16)
        c_bm.wait()
        c_ao = [cp(awoT_hbm.at[h], awoT.at[:, pl.ds(h * Dh, Dh)], bsem.at[3 * NP + H + h]) for h in range(H)]

        def body(h, mem):
            state = [mem]
            ga, gp = a_streams(h)
            interleave(ga, gp, b_steps(2 * (h - 2 * NA), 2, state), 8704.0, 12800.0, 3 * (S // PC) // 6)
            return state[0]

        mem = lax.fori_loop(2 * NA, H, body, memb[...].astype(F32))
        for c in c_ao:
            c.wait()
        RT = S // NT

        def out_copy(t):
            rows = pl.ds(pl.multiple_of(t * RT, RT), RT)
            return pltpu.make_async_copy(obuf.at[rows, :], out_hbm.at[0, rows, :], osem.at[t])

        def body_t(t, mem):
            state = [mem]

            def oproj():
                r0 = pl.multiple_of(t * RT, RT)
                accs = None
                for g in range(8):
                    cs = slice(g * HD // 8, (g + 1) * HD // 8)
                    tt = _nt(awoT[:, cs], ctx[pl.ds(r0, RT), cs])
                    accs = tt if accs is None else accs + tt
                    yield RT * 5
                obuf[pl.ds(r0, RT), :Dm] = accs.T.astype(BF16)

            g = oproj()
            gb = b_steps(S // SEG - NT + t, 1, state)
            n = 0
            for c in gb:
                n += 1
                if c is None or n % 3 == 0:
                    next(g, None)
            _drain(g)

            @pl.when(t < NT - 1)
            def _():
                out_copy(t).start()
            return state[0]

        lax.fori_loop(0, NT, body_t, mem)
        out_copy(NT - 1).start()
        for t in range(NT):
            out_copy(t).wait()

    scratch = [
        pltpu.VMEM((Dm, S), BF16), pltpu.VMEM((Dm, S), BF16), pltpu.VMEM((S, Dc), BF16),
        pltpu.VMEM((3, Dm + 2 * Dc, Dh), U32), pltpu.VMEM((3, NP, Dm, Dh), U32), pltpu.VMEM((M, Dm), BF16),
        pltpu.VMEM((S, Dm), BF16), pltpu.VMEM((Dm, Dh), BF16), pltpu.VMEM((Dc, Dh), BF16),
        pltpu.VMEM((Dc, Dh), BF16), pltpu.VMEM((Dm, HD), BF16), pltpu.VMEM((S, HD), BF16),
        pltpu.VMEM((S, Dm), F32), pltpu.VMEM((Dm, HD), BF16), pltpu.VMEM((Dm, HD), BF16),
        pltpu.VMEM((Dm, HD), BF16), pltpu.VMEM((Dm, HD), BF16), pltpu.VMEM((HD, Dm), BF16),
        pltpu.VMEM((S, 2 * Dm), BF16),
        *[pltpu.VMEM((2, S, Dh), BF16) for _ in range(3)],
        pltpu.SemaphoreType.DMA((8,)), pltpu.SemaphoreType.DMA((3, 3)),
        pltpu.SemaphoreType.DMA((3 * NP + 2 * H,)), pltpu.SemaphoreType.DMA((NT,)),
    ]
    return kernel, scratch


@functools.partial(jax.jit, static_argnames=("B_seg_len",))
def pallas_concat_heads__compressed_kv_cla__memory_aug_recurrent_mem_tr__prompt_kernel(
    A_x, A_c_kv, A_w_q, A_w_uk, A_w_uv, A_w_o,
    B_x, B_mem0, B_Wq, B_Wk, B_Wv, B_Wo, B_seg_len,
):
    B, S, Dm = A_x.shape
    Dc = A_c_kv.shape[-1]
    H, Dh = A_w_q.shape[1], A_w_q.shape[2]
    M = B_mem0.shape[1]
    SEG = int(B_seg_len)
    assert B == 1 and S == 2 * H * SEG
    kernel, scratch = _make_kernel(S, Dm, H, Dh, Dc, M, SEG)
    hbm = pl.BlockSpec(memory_space=pl.ANY)
    return pl.pallas_call(
        kernel,
        out_shape=jax.ShapeDtypeStruct((B, S, 2 * Dm), A_x.dtype),
        in_specs=[hbm] * 12,
        out_specs=hbm,
        scratch_shapes=scratch,
        compiler_params=pltpu.CompilerParams(vmem_limit_bytes=124 * 2 ** 20),
        name="cla_rmt",
    )(
        jnp.swapaxes(A_x, 1, 2), A_c_kv, A_w_q, A_w_uk, A_w_uv, jnp.swapaxes(A_w_o, 1, 2),
        jnp.swapaxes(B_x, 1, 2), B_mem0, B_Wq, B_Wk, B_Wv, jnp.swapaxes(B_Wo, 1, 2),
    )
```

```python
import functools

import jax
import jax.numpy as jnp
from jax import lax
import jax.experimental.pallas as pl
import jax.experimental.pallas.tpu as pltpu

F32 = jnp.float32
BF16 = jnp.bfloat16
U32 = jnp.uint32
LOG2E = 1.4426950408889634
NEG = -1e30


def _nn(a, b):
    return jnp.dot(a, b, preferred_element_type=F32)


def _nt(a, b):
    return lax.dot_general(a, b, (((1,), (1,)), ((), ())), preferred_element_type=F32)


def _half(u, odd):
    if isinstance(odd, bool):
        bits = (u & jnp.uint32(0xFFFF0000)) if odd else (u << 16)
    else:
        bits = jnp.where(odd, u, u << 16) & jnp.uint32(0xFFFF0000)
    return pltpu.bitcast(bits, F32).astype(BF16)


def _drain(*gens):
    for g in gens:
        for _ in g:
            pass


def _make_kernel(S, Dm, H, Dh, Dc, M, SEG, BQ=256, G=4, PC=256, NA=2):
    L = M + SEG
    HD = H * Dh
    NP = H // 2
    NT = 4 * NA
    assert (NT - 1) * (S // NT) <= S - NT * SEG
    qscale = Dh ** -0.5 * LOG2E
    KW = (Dm, Dc, Dc)
    KO = (0, Dm, Dm + Dc)

    def kernel(axT_hbm, ac_hbm, awq_hbm, awk_hbm, awv_hbm, awoT_hbm,
               bxT_hbm, bmem_hbm, bwq_hbm, bwk_hbm, bwv_hbm, bwoT_hbm,
               out_hbm,
               xTa, xTb, ac, araw, braw, memb, ax, awq, awk, awv, awoT, ctx,
               bx32, bwq, bwk, bwv, bwoT, bwo, obuf, qs, ks, vs, sems, asem, bsem, osem):
        aw32 = [w.bitcast(U32) for w in (awq_hbm, awk_hbm, awv_hbm)]
        bw32 = [w.bitcast(U32) for w in (bwq_hbm, bwk_hbm, bwv_hbm)]

        def a_wcopies(p, b):
            return [pltpu.make_async_copy(aw32[i].at[:, p, :], araw.at[b, pl.ds(KO[i], KW[i]), :], asem.at[b, i])
                    for i in range(3)]

        def cp(src, dst, sem):
            c = pltpu.make_async_copy(src, dst, sem)
            c.start()
            return c

        c_ax = cp(axT_hbm.at[0], xTa, sems.at[0])
        c_ac = cp(ac_hbm.at[0], ac, sems.at[1])
        for p in range(2):
            for c in a_wcopies(p, p):
                c.start()
        TC = 256
        c_ax.wait()
        for i in range(S // TC):
            ax[i * TC:(i + 1) * TC, :] = xTa[:, i * TC:(i + 1) * TC].astype(F32).T.astype(BF16)
        c_ac.wait()
        for c in a_wcopies(0, 0):
            c.wait()
        c_bw = [[cp(bw32[i].at[:, p, :], braw.at[i, p], bsem.at[i * NP + p]) for p in range(NP)] for i in range(3)]
        c_bx = cp(bxT_hbm.at[0], xTb, sems.at[2])
        c_bm = cp(bmem_hbm.at[0], memb, sems.at[3])
        c_bo = [cp(bwoT_hbm.at[h], bwoT.at[:, pl.ds(h * Dh, Dh)], bsem.at[3 * NP + h]) for h in range(H)]

        def a_proj(b, odd, slot):
            awq[...] = _half(araw[b, KO[0]:KO[0] + KW[0], :], odd)
            awk[...] = _half(araw[b, KO[1]:KO[1] + KW[1], :], odd)
            awv[...] = _half(araw[b, KO[2]:KO[2] + KW[2], :], odd)
            for r in range(S // PC):
                rs = slice(r * PC, (r + 1) * PC)
                qs[slot, rs, :] = (_nn(ax[rs, :], awq[...]) * qscale).astype(BF16)
                yield PC * 5 // 4
                ks[slot, rs, :] = _nn(ac[rs, :], awk[...]).astype(BF16)
                yield PC
                vs[slot, rs, :] = _nn(ac[rs, :], awv[...]).astype(BF16)
                yield PC

        def a_attn(h, slot):
            cs = pl.ds(pl.multiple_of(h * Dh, Dh), Dh)
            row = lax.broadcasted_iota(jnp.int32, (128, 128), 0)
            col = lax.broadcasted_iota(jnp.int32, (128, 128), 1)
            tri = row >= col
            nsub = BQ // 128

            def scores(i):
                qi = qs[slot, i * BQ:(i + 1) * BQ, :]
                pre = _nt(qi, ks[slot, 0:i * BQ, :]) if i > 0 else None
                res = []
                for a in range(nsub):
                    parts = [pre[a * 128:(a + 1) * 128]] if i > 0 else []
                    qa = qi[a * 128:(a + 1) * 128]
                    if a > 0:
                        parts.append(_nt(qa, ks[slot, i * BQ:i * BQ + a * 128, :]))
                    sd = _nt(qa, ks[slot, i * BQ + a * 128:i * BQ + (a + 1) * 128, :])
                    parts.append(jnp.where(tri, sd, NEG))
                    res.append(jnp.concatenate(parts, axis=1) if len(parts) > 1 else parts[0])
                return res

            nb = S // BQ
            cur = scores(0)
            yield 32 * nsub * (nsub + 1) // 2
            for i in range(nb):
                nxt = None
                if i + 1 < nb:
                    nxt = scores(i + 1)
                    yield BQ * (i + 1) * nsub // 4 + 32 * nsub * (nsub + 1) // 2
                for a in range(nsub):
                    sc = cur[a]
                    m = jnp.max(sc, axis=1, keepdims=True)
                    p = jnp.exp2(sc - m)
                    l = jnp.sum(p, axis=1, keepdims=True)
                    o = _nn(p.astype(BF16), vs[slot, 0:i * BQ + (a + 1) * 128, :])
                    r0 = i * BQ + a * 128
                    ctx[r0:r0 + 128, cs] = (o * pltpu.reciprocal(l, approx=True)).astype(BF16)
                    yield 32 * (i * nsub + a + 1)
                cur = nxt

        rowb = lax.broadcasted_iota(jnp.int32, (L, L), 0)
        colb = lax.broadcasted_iota(jnp.int32, (L, L), 1)
        maskb = (rowb < M) | (rowb >= colb)
        NG = H // G
        GW = G * Dh

        def b_steps(s0, n, state):
            for s in range(n):
                r0 = pl.multiple_of((s0 + s) * SEG, SEG)
                hh = jnp.concatenate([state[0], bx32[pl.ds(r0, SEG), :]], axis=0)
                qkv = []
                for g in range(NG):
                    cs = slice(g * GW, (g + 1) * GW)
                    q = _nn(hh, bwq[:, cs]) * qscale
                    k = _nn(hh, bwk[:, cs]).astype(BF16)
                    v = _nn(hh, bwv[:, cs]).astype(BF16)
                    qkv.append((q, k, v))
                    yield 3 * 5 * G * L // 4
                scs = []
                for g in range(NG):
                    q, k, v = qkv[g]
                    for j in range(G):
                        hs = slice(j * Dh, (j + 1) * Dh)
                        scs.append(jnp.where(maskb, _nt(q[:, hs], k[:, hs]), NEG))
                yield None
                ps = []
                for sc in scs:
                    m = jnp.max(sc, axis=-1, keepdims=True)
                    p = jnp.exp2(sc - m)
                    l = jnp.sum(p, axis=-1, keepdims=True)
                    ps.append((p, pltpu.reciprocal(l, approx=True)))
                yield None
                att = []
                for g in range(NG):
                    v = qkv[g][2]
                    outs = [_nn(ps[g * G + j][0], v[:, j * Dh:(j + 1) * Dh]) * ps[g * G + j][1] for j in range(G)]
                    att.append(jnp.concatenate(outs, axis=1) if G > 1 else outs[0])
                yield None
                o = None
                for g in range(NG):
                    t = _nn(att[g], bwo[g * GW:(g + 1) * GW, :])
                    o = t if o is None else o + t
                    yield 5 * G * L // 4
                yield None
                obuf[pl.ds(r0, SEG), Dm:] = o[M:].astype(BF16)
                state[0] = o[:M].astype(BF16).astype(F32)

        def interleave(ga, gp, gb, ta, tb, nfill):
            da = db = 0.0
            a_alive = True
            stage = 0
            for c in gb:
                if c is None:
                    for _ in range(nfill[stage % 4]):
                        next(gp, None)
                    stage += 1
                    continue
                db += c
                while a_alive and da / ta < db / tb:
                    ca = next(ga, None)
                    if ca is None:
                        a_alive = False
                    else:
                        da += ca
            _drain(ga, gp)

        def a_streams(h):
            @pl.when((h % 2 == 0) & (h // 2 + 2 < NP))
            def _():
                for c in a_wcopies(h // 2 + 2, (h // 2 + 2) % 3):
                    c.start()

            @pl.when((h % 2 == 1) & ((h + 1) // 2 < NP))
            def _():
                for c in a_wcopies((h + 1) // 2, ((h + 1) // 2) % 3):
                    c.wait()
            hn = jnp.minimum(h + 1, H - 1)
            return a_attn(h, h % 2), a_proj((hn // 2) % 3, hn % 2 == 1, (h + 1) % 2)

        _drain(a_proj(0, False, 0))

        def body_a(h, carry):
            ga, gp = a_streams(h)
            interleave(ga, iter(()), gp, 8704.0, 6656.0, 0)
            return carry

        lax.fori_loop(0, 2 * NA, body_a, 0)

        for i, dst in enumerate((bwq, bwk, bwv)):
            for p in range(NP):
                c_bw[i][p].wait()
                u = braw[i, p]
                dst[:, (2 * p) * Dh:(2 * p + 1) * Dh] = _half(u, False)
                dst[:, (2 * p + 1) * Dh:(2 * p + 2) * Dh] = _half(u, True)
        c_bx.wait()
        for i in range(S // TC):
            bx32[i * TC:(i + 1) * TC, :] = xTb[:, i * TC:(i + 1) * TC].astype(F32).T
        for c in c_bo:
            c.wait()
        for h in range(H):
            bwo[h * Dh:(h + 1) * Dh, :] = bwoT[:, h * Dh:(h + 1) * Dh].astype(F32).T.astype(BF16)
        c_bm.wait()
        c_ao = [cp(awoT_hbm.at[h], awoT.at[:, pl.ds(h * Dh, Dh)], bsem.at[3 * NP + H + h]) for h in range(H)]

        def body(h, mem):
            state = [mem]
            ga, gp = a_streams(h)
            interleave(ga, gp, b_steps(2 * (h - 2 * NA), 2, state), 8704.0, 12800.0, (1, 4, 3, 4))
            return state[0]

        mem = lax.fori_loop(2 * NA, H, body, memb[...].astype(F32))
        for c in c_ao:
            c.wait()
        RT = S // NT

        def out_copy(t):
            rows = pl.ds(pl.multiple_of(t * RT, RT), RT)
            return pltpu.make_async_copy(obuf.at[rows, :], out_hbm.at[0, rows, :], osem.at[t])

        def body_t(t, mem):
            state = [mem]

            def oproj():
                r0 = pl.multiple_of(t * RT, RT)
                accs = None
                for g in range(8):
                    cs = slice(g * HD // 8, (g + 1) * HD // 8)
                    tt = _nt(awoT[:, cs], ctx[pl.ds(r0, RT), cs])
                    accs = tt if accs is None else accs + tt
                    yield RT * 5
                obuf[pl.ds(r0, RT), :Dm] = accs.T.astype(BF16)

            g = oproj()
            gb = b_steps(S // SEG - NT + t, 1, state)
            n = 0
            for c in gb:
                n += 1
                if c is None or n % 3 == 0:
                    next(g, None)
            _drain(g)

            @pl.when(t < NT - 1)
            def _():
                out_copy(t).start()
            return state[0]

        lax.fori_loop(0, NT, body_t, mem)
        out_copy(NT - 1).start()
        for t in range(NT):
            out_copy(t).wait()

    scratch = [
        pltpu.VMEM((Dm, S), BF16), pltpu.VMEM((Dm, S), BF16), pltpu.VMEM((S, Dc), BF16),
        pltpu.VMEM((3, Dm + 2 * Dc, Dh), U32), pltpu.VMEM((3, NP, Dm, Dh), U32), pltpu.VMEM((M, Dm), BF16),
        pltpu.VMEM((S, Dm), BF16), pltpu.VMEM((Dm, Dh), BF16), pltpu.VMEM((Dc, Dh), BF16),
        pltpu.VMEM((Dc, Dh), BF16), pltpu.VMEM((Dm, HD), BF16), pltpu.VMEM((S, HD), BF16),
        pltpu.VMEM((S, Dm), F32), pltpu.VMEM((Dm, HD), BF16), pltpu.VMEM((Dm, HD), BF16),
        pltpu.VMEM((Dm, HD), BF16), pltpu.VMEM((Dm, HD), BF16), pltpu.VMEM((HD, Dm), BF16),
        pltpu.VMEM((S, 2 * Dm), BF16),
        *[pltpu.VMEM((2, S, Dh), BF16) for _ in range(3)],
        pltpu.SemaphoreType.DMA((8,)), pltpu.SemaphoreType.DMA((3, 3)),
        pltpu.SemaphoreType.DMA((3 * NP + 2 * H,)), pltpu.SemaphoreType.DMA((NT,)),
    ]
    return kernel, scratch


@functools.partial(jax.jit, static_argnames=("B_seg_len",))
def pallas_concat_heads__compressed_kv_cla__memory_aug_recurrent_mem_tr__prompt_kernel(
    A_x, A_c_kv, A_w_q, A_w_uk, A_w_uv, A_w_o,
    B_x, B_mem0, B_Wq, B_Wk, B_Wv, B_Wo, B_seg_len,
):
    B, S, Dm = A_x.shape
    Dc = A_c_kv.shape[-1]
    H, Dh = A_w_q.shape[1], A_w_q.shape[2]
    M = B_mem0.shape[1]
    SEG = int(B_seg_len)
    assert B == 1 and S == 2 * H * SEG
    kernel, scratch = _make_kernel(S, Dm, H, Dh, Dc, M, SEG)
    hbm = pl.BlockSpec(memory_space=pl.ANY)
    return pl.pallas_call(
        kernel,
        out_shape=jax.ShapeDtypeStruct((B, S, 2 * Dm), A_x.dtype),
        in_specs=[hbm] * 12,
        out_specs=hbm,
        scratch_shapes=scratch,
        compiler_params=pltpu.CompilerParams(vmem_limit_bytes=124 * 2 ** 20),
        name="cla_rmt",
    )(
        jnp.swapaxes(A_x, 1, 2), A_c_kv, A_w_q, A_w_uk, A_w_uv, jnp.swapaxes(A_w_o, 1, 2),
        jnp.swapaxes(B_x, 1, 2), B_mem0, B_Wq, B_Wk, B_Wv, jnp.swapaxes(B_Wo, 1, 2),
    )
```
